```python
import jax
import jax.numpy as jnp

def _softmax(x, axis=-1):
    return jax.nn.softmax(x, axis=axis)
def _gelu(x):
    return jax.nn.gelu(x, approximate=True)
def _silu(x):
    return jax.nn.silu(x)
def _sigmoid(x):
    return jax.nn.sigmoid(x)
def _layernorm(x, axis=-1, eps=1e-5):
    m = jnp.mean(x, axis=axis, keepdims=True)
    v = jnp.var(x, axis=axis, keepdims=True)
    return (x - m) / jnp.sqrt(v + eps)
def _scatter_add(tgt, idx, src, axis=0):
    return tgt.at[idx].add(src)
def _segment_sum(src, seg, n):
    return jax.ops.segment_sum(src, seg, n)
class _Rng:
    def __init__(self, key):
        self._k = key
    def _next(self):
        self._k, sub = jax.random.split(self._k)
        return sub
    def normal(self, shape):
        return jax.random.normal(self._next(), shape, dtype=jnp.bfloat16)
    def randint(self, lo, hi, shape):
        return jax.random.randint(self._next(), shape, lo, hi, dtype=jnp.int32)
    def uniform(self, shape, lo=0.0, hi=1.0):
        return jax.random.uniform(self._next(), shape, jnp.bfloat16, lo, hi)
    def permutation(self, n):
        return jax.random.permutation(self._next(), n)


kernel_name = 'gated_mix__compressed_kv_cla__ssm_conv_h3__prompt'

def setup_inputs():
    _rng = _Rng(jax.random.key(int.from_bytes(__import__("os").urandom(4), "little")))
    _w = (lambda a: (lambda t: t.astype(jnp.bfloat16) if jnp.issubdtype(t.dtype, jnp.floating) else t)(jnp.asarray(a)))
    def _A_setup():
        B, H, Sq, Sk, D, M = 1, 32, 2048, 2048, 128, 1024
        Dc = 4 * D
        return {
            "x": _w((lambda *s: _rng.normal(s) * 0.05)(B, Sq, M)),
            "c_kv": _w((lambda *s: _rng.normal(s) * 0.05)(B, Sk, Dc)),
            "w_q": _w((lambda *s: _rng.normal(s) * 0.05)(M, H, D) * (M ** -0.5)),
            "w_uk": _w((lambda *s: _rng.normal(s) * 0.05)(Dc, H, D) * (Dc ** -0.5)),
            "w_uv": _w((lambda *s: _rng.normal(s) * 0.05)(Dc, H, D) * (Dc ** -0.5)),
            "w_o": _w((lambda *s: _rng.normal(s) * 0.05)(H, D, M) * ((H * D) ** -0.5)),
        }
    _A_in = _A_setup()

    def _B_setup():
        B, S, D = 1, 2048, 1024
        ks = 4
        return {
            "q": _w((lambda *s: _rng.normal(s) * 0.05)(B, S, D)),
            "k": _w((lambda *s: _rng.normal(s) * 0.05)(B, S, D)),
            "v": _w((lambda *s: _rng.normal(s) * 0.05)(B, S, D)),
            "shift_k": _w((lambda *s: _rng.normal(s) * 0.05)(D, ks) * 0.5),
            "ssm_k": _w((lambda *s: _rng.normal(s) * 0.05)(D, S) * (1.0 / S ** 0.5)),
            "ssm_D": _w((lambda *s: _rng.normal(s) * 0.05)(D)),
        }
    _B_in = _B_setup()

    return {
        "A_x": _A_in["x"],
        "A_c_kv": _A_in["c_kv"],
        "A_w_q": _A_in["w_q"],
        "A_w_uk": _A_in["w_uk"],
        "A_w_uv": _A_in["w_uv"],
        "A_w_o": _A_in["w_o"],
        "B_q": _B_in["q"],
        "B_k": _B_in["k"],
        "B_v": _B_in["v"],
        "B_shift_k": _B_in["shift_k"],
        "B_ssm_k": _B_in["ssm_k"],
        "B_ssm_D": _B_in["ssm_D"],
        "gate_w": _w((lambda *s: _rng.normal(s) * 0.05)(1024)),
    }

def reference(A_x, A_c_kv, A_w_q, A_w_uk, A_w_uv, A_w_o, B_q, B_k, B_v, B_shift_k, B_ssm_k, B_ssm_D, gate_w):
    def _A_ref(x, c_kv, w_q, w_uk, w_uv, w_o):
        B, Sq, M = x.shape[0], x.shape[1], x.shape[2]
        Sk = c_kv.shape[1]
        H, D = w_q.shape[1], w_q.shape[2]
        q = jnp.einsum("bqm,mhd->bhqd", x, w_q)
        k = jnp.einsum("bkc,chd->bhkd", c_kv, w_uk)
        v = jnp.einsum("bkc,chd->bhkd", c_kv, w_uv)
        scores = jnp.einsum("bhqd,bhkd->bhqk", q, k) * (D ** -0.5)
        off = Sk - Sq
        qi = jnp.arange(Sq)[:, None]
        kj = jnp.arange(Sk)[None, :]
        cmask = kj <= (qi + off)
        scores = jnp.where(cmask[None, None], scores, -1e9)
        p = _softmax(scores, axis=-1)
        ctx = jnp.einsum("bhqk,bhkd->bhqd", p, v)
        return jnp.einsum("bhqd,hdm->bqm", ctx, w_o)

    def _B_ref(q, k, v, shift_k, ssm_k, ssm_D):
        B, S, D = q.shape
        ks = shift_k.shape[-1]
        k_pad = jnp.pad(k, ((0, 0), (ks - 1, 0), (0, 0)))
        k_shift = jnp.zeros_like(k)
        for t in range(ks):
            k_shift = k_shift + k_pad[:, t:t + S, :] * shift_k[:, ks - 1 - t][None, None, :]
        kv = k_shift * v
        L = 2 * S
        kv_pad = jnp.pad(kv, ((0, 0), (0, S), (0, 0)))
        kf_pad = jnp.pad(ssm_k, ((0, 0), (0, S)))
        kv_f = (lambda x, axes=(-2,-1): jnp.fft.rfft2(x.astype(jnp.float32), axes=axes))(kv_pad[:, None, :, :], axes=(1, 2))
        kf_f = (lambda x, axes=(-2,-1): jnp.fft.rfft2(x.astype(jnp.float32), axes=axes))(kf_pad[:, None, :], axes=(1, 2))
        kf_f = (lambda x, *d: x.transpose(*d))(kf_f, 1, 2, 0)
        y_f = kv_f * kf_f[None, :, :, :]
        y = (lambda x, s, axes=(-2,-1): jnp.fft.irfft2(x, s=s, axes=axes).astype(jnp.bfloat16))(y_f, (1, L), axes=(1, 2))[:, 0, :S, :]
        y = y + kv * ssm_D[None, None, :]
        return q * y

    x = A_x
    g = _sigmoid((x * gate_w).sum(-1, keepdims=True))
    a = _A_ref(x, A_c_kv, A_w_q, A_w_uk, A_w_uv, A_w_o)
    b = _B_ref(x, B_k, B_v, B_shift_k, B_ssm_k, B_ssm_D)
    return g * a + (1 - g) * b
```

```python
import numpy as np
import jax
import jax.numpy as jnp
import jax.experimental.pallas as pl
import jax.experimental.pallas.tpu as pltpu

P = 128
BQ = 256
F32, BF16 = jnp.float32, jnp.bfloat16


def _dft():
    f = np.concatenate([np.arange(0, P, 2), np.arange(1, P, 2)])
    w = 2 * np.pi * (f[:, None] + 0.5) * np.arange(P)[None, :] / (2 * P)
    fwd = np.concatenate([np.cos(w), -np.sin(w)], 0)
    inv = np.concatenate([np.cos(w).T, -np.sin(w).T], 1) / P
    return fwd.astype(np.float32), inv.astype(np.float32)


def _mm(a, b):
    return jnp.dot(a, b, preferred_element_type=F32)


def _mmt(a, b):
    return jax.lax.dot_general(a, b, (((1,), (1,)), ((), ())), preferred_element_type=F32)


def _kernel(x_ref, c_ref, wq_ref, wk_ref, wv_ref, wo_ref, bk_ref, bv_ref, sh_ref,
            ssm_ref, d_ref, gw_ref, fwd_ref, inv_ref, o_ref,
            acc, b_s, k_s, v_s, xf, kf, z_s, kv_s, kp_s):
    h = pl.program_id(0)
    H = pl.num_programs(0)
    S, M = x_ref.shape
    D = wq_ref.shape[1]
    NB = S // P
    G = H * 128 // M
    ks = sh_ref.shape[0]

    @pl.when(h == 0)
    def _():
        acc[...] = jnp.zeros_like(acc)
        kp_s[0:8, :] = jnp.zeros((8, 128), F32)

    @pl.when(h % G == 0)
    def _():
        kp_s[8:, :] = bk_ref[...].astype(F32)
        sh = sh_ref[...].astype(F32)
        fw = fwd_ref[...]
        for i in range(NB):
            t = sum(kp_s[8 + i * P - j:8 + (i + 1) * P - j, :] * sh[j:j + 1] for j in range(ks))
            kv = (t.astype(BF16).astype(F32) * bv_ref[i * P:(i + 1) * P, :].astype(F32)).astype(BF16)
            kv_s[i * P:(i + 1) * P, :] = kv
            xf[i] = _mm(fw, kv)
            kf[i] = _mmt(fw, ssm_ref[:, i * P:(i + 1) * P])

    def mac(r):
        re, im = pl.ds(r, 8), pl.ds(P + r, 8)
        sg = jnp.where(r < P // 2, 1.0, -1.0).astype(F32)
        T = 4
        prev = None
        for i0 in range(0, NB, T):
            zr = [None] * T
            zi = [None] * T
            for m in range(i0 + T):
                c, d = kf[m, re, :], kf[m, im, :]
                for u in range(T):
                    j = i0 + u - m
                    if j < 0:
                        continue
                    a, b = xf[j, re, :], xf[j, im, :]
                    pr, pi = a * c - b * d, a * d + b * c
                    zr[u] = pr if zr[u] is None else zr[u] + pr
                    zi[u] = pi if zi[u] is None else zi[u] + pi
            for u in range(T):
                r_, i_ = zr[u], zi[u]
                if prev is not None:
                    r_, i_ = r_ - sg * prev[1], i_ + sg * prev[0]
                prev = (zr[u], zi[u])
                z_s[i0 + u, re, :] = r_
                z_s[i0 + u, im, :] = i_

    scale = np.float32(D ** -0.5 * np.log2(np.e))
    NQ = S // BQ
    NM = P // 8 // G

    def proj(i):
        r = slice(i * BQ, (i + 1) * BQ)
        c = c_ref[r, :]
        k_s[r, :] = _mm(c, wk_ref[...]).astype(BF16)
        v_s[r, :] = _mm(c, wv_ref[...]).astype(BF16)
        return (_mm(x_ref[r, :], wq_ref[...]) * scale).astype(BF16)

    row = jax.lax.broadcasted_iota(jnp.int32, (BQ, BQ), 0)
    col = jax.lax.broadcasted_iota(jnp.int32, (BQ, BQ), 1)
    q = proj(0)
    for i in range(NQ):
        r = slice(i * BQ, (i + 1) * BQ)
        sd = jnp.where(col <= row, _mmt(q, k_s[r, :]), -1e9)
        s = jnp.concatenate([_mmt(q, k_s[0:i * BQ, :]), sd], 1) if i else sd
        if i + 1 < NQ:
            q = proj(i + 1)
        if i % (NQ // NM) == 1:
            mac(pl.multiple_of(((h % G) * NM + i // (NQ // NM)) * 8, 8))
        p = jnp.exp2(s - jnp.max(s, axis=1, keepdims=True))
        l = jnp.sum(p, axis=1, keepdims=True)
        ctx = (_mm(p.astype(BF16), v_s[0:(i + 1) * BQ, :]) * (1.0 / l)).astype(BF16)
        acc[r, :] += _mm(ctx, wo_ref[...])

    @pl.when(h % G == G - 1)
    def _():
        iv = inv_ref[...]
        dd = d_ref[...].astype(F32)
        cs = pl.ds(pl.multiple_of((h // G) * 128, 128), 128)
        for i in range(NB):
            r = slice(i * P, (i + 1) * P)
            y = _mm(iv, z_s[i].astype(BF16)) + kv_s[r, :].astype(F32) * dd
            b_s[r, cs] = x_ref[r, cs].astype(F32) * y

    @pl.when(h == H - 1)
    def _():
        gw = gw_ref[...].astype(F32)
        for i in range(NQ):
            r = slice(i * BQ, (i + 1) * BQ)
            g = jax.nn.sigmoid(jnp.sum(x_ref[r, :].astype(F32) * gw, axis=1, keepdims=True))
            o_ref[r, :] = (g * acc[r, :] + (1 - g) * b_s[r, :]).astype(o_ref.dtype)


@jax.jit
def pallas_gated_mix__compressed_kv_cla__ssm_conv_h3__prompt_kernel(
    A_x, A_c_kv, A_w_q, A_w_uk, A_w_uv, A_w_o, B_q, B_k, B_v, B_shift_k, B_ssm_k, B_ssm_D, gate_w,
):
    _, S, M = A_x.shape
    C = A_c_kv.shape[2]
    _, H, D = A_w_q.shape
    G = H * 128 // M
    ks = B_shift_k.shape[1]
    fwd, inv = _dft()
    full = lambda *s: pl.BlockSpec(s, lambda h: (0,) * len(s))
    hd = lambda n: pl.BlockSpec((n, D), lambda h: (0, h))
    ch = lambda n: pl.BlockSpec((n, 128), lambda h: (0, h // G))
    NB = S // P
    out = pl.pallas_call(
        _kernel,
        grid=(H,),
        in_specs=[full(S, M), full(S, C), hd(M), hd(C), hd(C),
                  pl.BlockSpec((None, D, M), lambda h: (h, 0, 0)),
                  ch(S), ch(S), ch(ks),
                  pl.BlockSpec((128, S), lambda h: (h // G, 0)),
                  ch(1), full(1, M), full(2 * P, P), full(P, 2 * P)],
        out_specs=full(S, M),
        out_shape=jax.ShapeDtypeStruct((S, M), A_x.dtype),
        scratch_shapes=[pltpu.VMEM((S, M), F32), pltpu.VMEM((S, M), F32),
                        pltpu.VMEM((S, D), BF16), pltpu.VMEM((S, D), BF16),
                        pltpu.VMEM((NB, 2 * P, 128), F32), pltpu.VMEM((NB, 2 * P, 128), F32),
                        pltpu.VMEM((NB, 2 * P, 128), F32), pltpu.VMEM((S, 128), BF16),
                        pltpu.VMEM((S + 8, 128), F32)],
        compiler_params=pltpu.CompilerParams(dimension_semantics=("arbitrary",),
                                             vmem_limit_bytes=100 * 1024 * 1024),
    )(A_x[0], A_c_kv[0], A_w_q.reshape(M, H * D), A_w_uk.reshape(C, H * D), A_w_uv.reshape(C, H * D),
      A_w_o, B_k[0], B_v[0], B_shift_k.T, B_ssm_k, B_ssm_D.reshape(1, M), gate_w.reshape(1, M),
      jnp.asarray(fwd, BF16), jnp.asarray(inv, BF16))
    return out[None]
```

```python
import numpy as np
import jax
import jax.numpy as jnp
import jax.experimental.pallas as pl
import jax.experimental.pallas.tpu as pltpu

P = 128
BQ = 256
F32, BF16 = jnp.float32, jnp.bfloat16


def _dft():
    f = np.concatenate([np.arange(0, P, 2), np.arange(1, P, 2)])
    w = 2 * np.pi * (f[:, None] + 0.5) * np.arange(P)[None, :] / (2 * P)
    fwd = np.concatenate([np.cos(w), -np.sin(w)], 0)
    inv = np.concatenate([np.cos(w).T, -np.sin(w).T], 1) / P
    return fwd.astype(np.float32), inv.astype(np.float32)


def _mm(a, b):
    return jnp.dot(a, b, preferred_element_type=F32)


def _mmt(a, b):
    return jax.lax.dot_general(a, b, (((1,), (1,)), ((), ())), preferred_element_type=F32)


def _kernel(x_ref, c_ref, wq_ref, wk_ref, wv_ref, wo_ref, bk_ref, bv_ref, sh_ref,
            ssm_ref, d_ref, gw_ref, fwd_ref, inv_ref, o_ref,
            acc, b_s, k_s, v_s, xf, kf, z_s, kv_s, kp_s, wq_s, wk_s, wv_s, wq_b, wk_b, wv_b, sem):
    h = pl.program_id(0)
    H = pl.num_programs(0)
    S, M = x_ref.shape
    D = wq_ref.shape[2]
    NB = S // P
    G = H * 128 // M
    ks = sh_ref.shape[0]

    @pl.when(h == 0)
    def _():
        acc[...] = jnp.zeros_like(acc)
        kp_s[0:8, :] = jnp.zeros((8, 128), F32)

    @pl.when(h % G == 0)
    def _():
        kp_s[8:, :] = bk_ref[...].astype(F32)
        sh = sh_ref[...].astype(F32)
        fw = fwd_ref[...]
        for i in range(NB):
            t = sum(kp_s[8 + i * P - j:8 + (i + 1) * P - j, :] * sh[j:j + 1] for j in range(ks))
            kv = (t.astype(BF16).astype(F32) * bv_ref[i * P:(i + 1) * P, :].astype(F32)).astype(BF16)
            kv_s[i * P:(i + 1) * P, :] = kv
            xf[i] = _mm(fw, kv)
            kf[i] = _mmt(fw, ssm_ref[:, i * P:(i + 1) * P])

    def mac(r):
        re, im = pl.ds(r, 8), pl.ds(P + r, 8)
        sg = jnp.where(r < P // 2, 1.0, -1.0).astype(F32)
        T = 4
        prev = None
        for i0 in range(0, NB, T):
            zr = [None] * T
            zi = [None] * T
            for m in range(i0 + T):
                c, d = kf[m, re, :], kf[m, im, :]
                for u in range(T):
                    j = i0 + u - m
                    if j < 0:
                        continue
                    a, b = xf[j, re, :], xf[j, im, :]
                    pr, pi = a * c - b * d, a * d + b * c
                    zr[u] = pr if zr[u] is None else zr[u] + pr
                    zi[u] = pi if zi[u] is None else zi[u] + pi
            for u in range(T):
                r_, i_ = zr[u], zi[u]
                if prev is not None:
                    r_, i_ = r_ - sg * prev[1], i_ + sg * prev[0]
                prev = (zr[u], zi[u])
                z_s[i0 + u, re, :] = r_
                z_s[i0 + u, im, :] = i_

    scale = np.float32(D ** -0.5 * np.log2(np.e))
    NQ = S // BQ
    NM = P // 8 // G

    def copies(p):
        return [pltpu.make_async_copy(w.bitcast(jnp.uint32).at[:, p, :], b.at[p % 2], sem.at[n])
                for n, (w, b) in enumerate(((wq_ref, wq_b), (wk_ref, wk_b), (wv_ref, wv_b)))]

    @pl.when(h == 0)
    def _():
        for cp in copies(0):
            cp.start()

    @pl.when(h % 2 == 0)
    def _():
        for cp in copies(h // 2):
            cp.wait()

        @pl.when(h + 2 < H)
        def _():
            for cp in copies(h // 2 + 1):
                cp.start()

    def head(w_b, dst):
        u = w_b[(h // 2) % 2]
        u = jnp.where(h % 2 == 0, u << 16, u & np.uint32(0xFFFF0000))
        dst[...] = pltpu.bitcast(u, F32).astype(BF16)

    head(wq_b, wq_s)
    head(wk_b, wk_s)
    head(wv_b, wv_s)

    def proj(i):
        r = slice(i * BQ, (i + 1) * BQ)
        c = c_ref[r, :]
        k_s[r, :] = _mm(c, wk_s[...]).astype(BF16)
        v_s[r, :] = _mm(c, wv_s[...]).astype(BF16)
        return (_mm(x_ref[r, :], wq_s[...]) * scale).astype(BF16)

    row = jax.lax.broadcasted_iota(jnp.int32, (BQ, BQ), 0)
    col = jax.lax.broadcasted_iota(jnp.int32, (BQ, BQ), 1)
    q = proj(0)
    for i in range(NQ):
        r = slice(i * BQ, (i + 1) * BQ)
        sd = jnp.where(col <= row, _mmt(q, k_s[r, :]), -1e9)
        s = jnp.concatenate([_mmt(q, k_s[0:i * BQ, :]), sd], 1) if i else sd
        if i + 1 < NQ:
            q = proj(i + 1)
        if i % (NQ // NM) == 1:
            mac(pl.multiple_of(((h % G) * NM + i // (NQ // NM)) * 8, 8))
        p = jnp.exp2(s - jnp.max(s, axis=1, keepdims=True))
        l = jnp.sum(p, axis=1, keepdims=True)
        ctx = (_mm(p.astype(BF16), v_s[0:(i + 1) * BQ, :]) * (1.0 / l)).astype(BF16)
        acc[r, :] += _mm(ctx, wo_ref[...])

    @pl.when(h % G == G - 1)
    def _():
        iv = inv_ref[...]
        dd = d_ref[...].astype(F32)
        cs = pl.ds(pl.multiple_of((h // G) * 128, 128), 128)
        for i in range(NB):
            r = slice(i * P, (i + 1) * P)
            y = _mm(iv, z_s[i].astype(BF16)) + kv_s[r, :].astype(F32) * dd
            b_s[r, cs] = x_ref[r, cs].astype(F32) * y

    @pl.when(h == H - 1)
    def _():
        gw = gw_ref[...].astype(F32)
        for i in range(NQ):
            r = slice(i * BQ, (i + 1) * BQ)
            g = jax.nn.sigmoid(jnp.sum(x_ref[r, :].astype(F32) * gw, axis=1, keepdims=True))
            o_ref[r, :] = (g * acc[r, :] + (1 - g) * b_s[r, :]).astype(o_ref.dtype)


@jax.jit
def pallas_gated_mix__compressed_kv_cla__ssm_conv_h3__prompt_kernel(
    A_x, A_c_kv, A_w_q, A_w_uk, A_w_uv, A_w_o, B_q, B_k, B_v, B_shift_k, B_ssm_k, B_ssm_D, gate_w,
):
    _, S, M = A_x.shape
    C = A_c_kv.shape[2]
    _, H, D = A_w_q.shape
    G = H * 128 // M
    ks = B_shift_k.shape[1]
    fwd, inv = _dft()
    full = lambda *s: pl.BlockSpec(s, lambda h: (0,) * len(s))
    hd = lambda n: pl.BlockSpec(memory_space=pl.ANY)
    ch = lambda n: pl.BlockSpec((n, 128), lambda h: (0, h // G))
    NB = S // P
    out = pl.pallas_call(
        _kernel,
        grid=(H,),
        in_specs=[full(S, M), full(S, C), hd(M), hd(C), hd(C),
                  pl.BlockSpec((None, D, M), lambda h: (h, 0, 0)),
                  ch(S), ch(S), ch(ks),
                  pl.BlockSpec((128, S), lambda h: (h // G, 0)),
                  ch(1), full(1, M), full(2 * P, P), full(P, 2 * P)],
        out_specs=full(S, M),
        out_shape=jax.ShapeDtypeStruct((S, M), A_x.dtype),
        scratch_shapes=[pltpu.VMEM((S, M), F32), pltpu.VMEM((S, M), F32),
                        pltpu.VMEM((S, D), BF16), pltpu.VMEM((S, D), BF16),
                        pltpu.VMEM((NB, 2 * P, 128), F32), pltpu.VMEM((NB, 2 * P, 128), F32),
                        pltpu.VMEM((NB, 2 * P, 128), F32), pltpu.VMEM((S, 128), BF16),
                        pltpu.VMEM((S + 8, 128), F32), pltpu.VMEM((M, D), BF16),
                        pltpu.VMEM((C, D), BF16), pltpu.VMEM((C, D), BF16),
                        pltpu.VMEM((2, M, D), jnp.uint32), pltpu.VMEM((2, C, D), jnp.uint32),
                        pltpu.VMEM((2, C, D), jnp.uint32), pltpu.SemaphoreType.DMA((3,))],
        compiler_params=pltpu.CompilerParams(dimension_semantics=("arbitrary",),
                                             vmem_limit_bytes=100 * 1024 * 1024),
    )(A_x[0], A_c_kv[0], A_w_q, A_w_uk, A_w_uv,
      A_w_o, B_k[0], B_v[0], B_shift_k.T, B_ssm_k, B_ssm_D.reshape(1, M), gate_w.reshape(1, M),
      jnp.asarray(fwd, BF16), jnp.asarray(inv, BF16))
    return out[None]
```

```python
import numpy as np
import jax
import jax.numpy as jnp
import jax.experimental.pallas as pl
import jax.experimental.pallas.tpu as pltpu

P = 128
BQ = 256
F32, BF16 = jnp.float32, jnp.bfloat16


def _dft():
    f = np.concatenate([np.arange(0, P, 2), np.arange(1, P, 2)])
    w = 2 * np.pi * (f[:, None] + 0.5) * np.arange(P)[None, :] / (2 * P)
    fwd = np.concatenate([np.cos(w), -np.sin(w)], 0)
    inv = np.concatenate([np.cos(w).T, -np.sin(w).T], 1) / P
    return fwd.astype(np.float32), inv.astype(np.float32)


def _mm(a, b):
    return jnp.dot(a, b, preferred_element_type=F32)


def _mmt(a, b):
    return jax.lax.dot_general(a, b, (((1,), (1,)), ((), ())), preferred_element_type=F32)


def _kernel(x_ref, c_ref, wq_ref, wk_ref, wv_ref, wo_ref, bk_ref, bv_ref, sh_ref,
            ssm_ref, d_ref, gw_ref, fwd_ref, inv_ref, o_ref,
            acc, b_s, k_s, v_s, xf, kf, z_s, kv_s, kp_s, wq_s, wk_s, wv_s, wq_b, wk_b, wv_b, sem):
    h = pl.program_id(0)
    H = pl.num_programs(0)
    S, M = x_ref.shape
    D = wq_ref.shape[2]
    NB = S // P
    G = H * 128 // M
    ks = sh_ref.shape[0]

    def copies(p):
        return [pltpu.make_async_copy(w.bitcast(jnp.uint32).at[:, p, :], b.at[p % 2], sem.at[n])
                for n, (w, b) in enumerate(((wq_ref, wq_b), (wk_ref, wk_b), (wv_ref, wv_b)))]

    def unpack(n):
        sft = ((1 - n % 2) * 16).astype(jnp.uint32)
        for w_b, dst in ((wk_b, wk_s), (wv_b, wv_s), (wq_b, wq_s)):
            u = (w_b[(n // 2) % 2] << sft) & np.uint32(0xFFFF0000)
            dst[...] = pltpu.bitcast(u, F32).astype(BF16)

    @pl.when(h == 0)
    def _():
        for cp in copies(h):
            cp.start()
        for cp in copies(h):
            cp.wait()
        unpack(h)

    @pl.when(h + 2 < H)
    def _():
        @pl.when(h % 2 == 0)
        def _():
            for cp in copies(h // 2 + 1):
                cp.start()

        @pl.when(h % 2 == 1)
        def _():
            for cp in copies(h // 2 + 1):
                cp.wait()

    @pl.when(h == 0)
    def _():
        acc[...] = jnp.zeros_like(acc)
        kp_s[0:8, :] = jnp.zeros((8, 128), F32)

    @pl.when(h % G == 0)
    def _():
        kp_s[8:, :] = bk_ref[...].astype(F32)
        sh = sh_ref[...].astype(F32)
        fw = fwd_ref[...]
        for i in range(NB):
            t = sum(kp_s[8 + i * P - j:8 + (i + 1) * P - j, :] * sh[j:j + 1] for j in range(ks))
            kv = (t.astype(BF16).astype(F32) * bv_ref[i * P:(i + 1) * P, :].astype(F32)).astype(BF16)
            kv_s[i * P:(i + 1) * P, :] = kv
            xf[i] = _mm(fw, kv)
            kf[i] = _mmt(fw, ssm_ref[:, i * P:(i + 1) * P])

    def mac(r):
        re, im = pl.ds(r, 8), pl.ds(P + r, 8)
        sg = jnp.where(r < P // 2, 1.0, -1.0).astype(F32)
        T = 4
        prev = None
        for i0 in range(0, NB, T):
            zr = [None] * T
            zi = [None] * T
            for m in range(i0 + T):
                c, d = kf[m, re, :], kf[m, im, :]
                for u in range(T):
                    j = i0 + u - m
                    if j < 0:
                        continue
                    a, b = xf[j, re, :], xf[j, im, :]
                    pr, pi = a * c - b * d, a * d + b * c
                    zr[u] = pr if zr[u] is None else zr[u] + pr
                    zi[u] = pi if zi[u] is None else zi[u] + pi
            for u in range(T):
                r_, i_ = zr[u], zi[u]
                if prev is not None:
                    r_, i_ = r_ - sg * prev[1], i_ + sg * prev[0]
                prev = (zr[u], zi[u])
                z_s[i0 + u, re, :] = r_
                z_s[i0 + u, im, :] = i_

    scale = np.float32(D ** -0.5 * np.log2(np.e))
    NQ = S // BQ
    NM = P // 8 // G

    def proj(i):
        r = slice(i * BQ, (i + 1) * BQ)
        c = c_ref[r, :]
        k_s[r, :] = _mm(c, wk_s[...]).astype(BF16)
        v_s[r, :] = _mm(c, wv_s[...]).astype(BF16)
        return (_mm(x_ref[r, :], wq_s[...]) * scale).astype(BF16)

    Hf = BQ // 2
    row = jax.lax.broadcasted_iota(jnp.int32, (Hf, Hf), 0)
    col = jax.lax.broadcasted_iota(jnp.int32, (Hf, Hf), 1)
    msk = lambda t: jnp.where(col <= row, t, -1e9)
    q = proj(0)
    for i in range(NQ):
        r = slice(i * BQ, (i + 1) * BQ)
        n0, n1 = i * BQ + Hf, (i + 1) * BQ
        s0 = _mmt(q, k_s[0:n0, :])
        s1 = msk(_mmt(q[Hf:], k_s[n0:n1, :]))
        st = msk(s0[:Hf, n0 - Hf:])
        st = jnp.concatenate([s0[:Hf, :n0 - Hf], st], 1) if i else st
        sb = s0[Hf:]
        if i % (NQ // NM) == 1:
            mac(pl.multiple_of(((h % G) * NM + i // (NQ // NM)) * 8, 8))
        mx = lambda t: jnp.max(t, axis=1, keepdims=True)
        sm = lambda t: jnp.sum(t, axis=1, keepdims=True)
        mb = mx(jnp.concatenate([sb, s1], 1))
        pt, pb, p1 = jnp.exp2(st - mx(st)), jnp.exp2(sb - mb), jnp.exp2(s1 - mb)
        if i + 1 < NQ:
            q = proj(i + 1)
        else:
            unpack(h + 1)
        o = _mm(jnp.concatenate([pt, pb], 0).astype(BF16), v_s[0:n0, :])
        ob = (o[Hf:] + _mm(p1.astype(BF16), v_s[n0:n1, :])) * (1.0 / sm(jnp.concatenate([pb, p1], 1)))
        ctx = jnp.concatenate([o[:Hf] * (1.0 / sm(pt)), ob], 0).astype(BF16)
        acc[r, :] += _mm(ctx, wo_ref[...])

    @pl.when(h % G == G - 1)
    def _():
        iv = inv_ref[...]
        dd = d_ref[...].astype(F32)
        cs = pl.ds(pl.multiple_of((h // G) * 128, 128), 128)
        for i in range(NB):
            r = slice(i * P, (i + 1) * P)
            y = _mm(iv, z_s[i].astype(BF16)) + kv_s[r, :].astype(F32) * dd
            b_s[r, cs] = x_ref[r, cs].astype(F32) * y

    @pl.when(h == H - 1)
    def _():
        gw = gw_ref[...].astype(F32)
        for i in range(NQ):
            r = slice(i * BQ, (i + 1) * BQ)
            g = jax.nn.sigmoid(jnp.sum(x_ref[r, :].astype(F32) * gw, axis=1, keepdims=True))
            o_ref[r, :] = (g * acc[r, :] + (1 - g) * b_s[r, :]).astype(o_ref.dtype)


@jax.jit
def pallas_gated_mix__compressed_kv_cla__ssm_conv_h3__prompt_kernel(
    A_x, A_c_kv, A_w_q, A_w_uk, A_w_uv, A_w_o, B_q, B_k, B_v, B_shift_k, B_ssm_k, B_ssm_D, gate_w,
):
    _, S, M = A_x.shape
    C = A_c_kv.shape[2]
    _, H, D = A_w_q.shape
    G = H * 128 // M
    ks = B_shift_k.shape[1]
    fwd, inv = _dft()
    full = lambda *s: pl.BlockSpec(s, lambda h: (0,) * len(s))
    hd = lambda n: pl.BlockSpec(memory_space=pl.ANY)
    ch = lambda n: pl.BlockSpec((n, 128), lambda h: (0, h // G))
    NB = S // P
    out = pl.pallas_call(
        _kernel,
        grid=(H,),
        in_specs=[full(S, M), full(S, C), hd(M), hd(C), hd(C),
                  pl.BlockSpec((None, D, M), lambda h: (h, 0, 0)),
                  ch(S), ch(S), ch(ks),
                  pl.BlockSpec((128, S), lambda h: (h // G, 0)),
                  ch(1), full(1, M), full(2 * P, P), full(P, 2 * P)],
        out_specs=full(S, M),
        out_shape=jax.ShapeDtypeStruct((S, M), A_x.dtype),
        scratch_shapes=[pltpu.VMEM((S, M), F32), pltpu.VMEM((S, M), F32),
                        pltpu.VMEM((S, D), BF16), pltpu.VMEM((S, D), BF16),
                        pltpu.VMEM((NB, 2 * P, 128), F32), pltpu.VMEM((NB, 2 * P, 128), F32),
                        pltpu.VMEM((NB, 2 * P, 128), F32), pltpu.VMEM((S, 128), BF16),
                        pltpu.VMEM((S + 8, 128), F32), pltpu.VMEM((M, D), BF16),
                        pltpu.VMEM((C, D), BF16), pltpu.VMEM((C, D), BF16),
                        pltpu.VMEM((2, M, D), jnp.uint32), pltpu.VMEM((2, C, D), jnp.uint32),
                        pltpu.VMEM((2, C, D), jnp.uint32), pltpu.SemaphoreType.DMA((3,))],
        compiler_params=pltpu.CompilerParams(dimension_semantics=("arbitrary",),
                                             vmem_limit_bytes=100 * 1024 * 1024),
    )(A_x[0], A_c_kv[0], A_w_q, A_w_uk, A_w_uv,
      A_w_o, B_k[0], B_v[0], B_shift_k.T, B_ssm_k, B_ssm_D.reshape(1, M), gate_w.reshape(1, M),
      jnp.asarray(fwd, BF16), jnp.asarray(inv, BF16))
    return out[None]
```
